```python
import os as _os
_os.environ.setdefault("JAX_PLATFORMS", "cpu")
import jax
import jax.numpy as jnp

def _softmax(x, axis=-1):
    return jax.nn.softmax(x, axis=axis)
def _gelu(x):
    return jax.nn.gelu(x, approximate=True)
def _silu(x):
    return jax.nn.silu(x)
def _sigmoid(x):
    return jax.nn.sigmoid(x)
def _layernorm(x, axis=-1, eps=1e-5):
    m = jnp.mean(x, axis=axis, keepdims=True)
    v = jnp.var(x, axis=axis, keepdims=True)
    return (x - m) / jnp.sqrt(v + eps)
def _scatter_add(tgt, idx, src, axis=0):
    return tgt.at[idx].add(src)
def _segment_sum(src, seg, n):
    return jax.ops.segment_sum(src, seg, n)
class _Rng:
    def __init__(self, key):
        self._k = key
    def _next(self):
        self._k, sub = jax.random.split(self._k)
        return sub
    def normal(self, shape):
        return jax.random.normal(self._next(), shape, dtype=jnp.bfloat16)
    def randint(self, lo, hi, shape):
        return jax.random.randint(self._next(), shape, lo, hi, dtype=jnp.int32)
    def uniform(self, shape, lo=0.0, hi=1.0):
        return jax.random.uniform(self._next(), shape, jnp.bfloat16, lo, hi)
    def permutation(self, n):
        return jax.random.permutation(self._next(), n)


kernel_name = 'gated_mix__softmax_full_mha__dense_activation_relu__prompt'

def setup_inputs():
    _rng = _Rng(jax.random.key(int.from_bytes(__import__("os").urandom(4), "little")))
    _w = (lambda a: (lambda t: t.astype(jnp.bfloat16) if jnp.issubdtype(t.dtype, jnp.floating) else t)(jnp.asarray(a)))
    def _A_setup():
        B, S, D = 1, 2048, 640
        return {
            "x": _w((lambda *s: _rng.normal(s) * 0.05)(B, S, D)),
            "wqkv": _w((lambda *s: _rng.normal(s) * 0.8)(D, 3 * D)),
            "wo": _w((lambda *s: _rng.normal(s) * 0.05)(D, D)),
        }
    _A_in = _A_setup()

    def _B_setup():
        B, S, D, Dff = 1, 2048, 640, 1536
        return {
            "x": _w((lambda *s: _rng.normal(s) * 0.05)(B, S, D)),
            "w1": _w((lambda *s: _rng.normal(s) * 0.05)(D, Dff)),
            "w2": _w((lambda *s: _rng.normal(s) * 0.05)(Dff, D)),
        }
    _B_in = _B_setup()

    return {
        "A_x": _A_in["x"],
        "A_wqkv": _A_in["wqkv"],
        "A_wo": _A_in["wo"],
        "B_x": _B_in["x"],
        "B_w1": _B_in["w1"],
        "B_w2": _B_in["w2"],
        "gate_w": _w((lambda *s: _rng.normal(s) * 0.05)(640) * 16.0),
    }

def reference(A_x, A_wqkv, A_wo, B_x, B_w1, B_w2, gate_w):
    def _A_ref(x, wqkv, wo):
        B, S, D = x.shape
        H = 32; Dh = D // H
        qkv = (lambda x, *d: x.transpose(*d))((x @ wqkv).reshape(B, S, 3, H, Dh), 2, 0, 3, 1, 4)
        q, k, v = qkv[0], qkv[1], qkv[2]
        scale = Dh ** -0.5
        scores = jnp.einsum("bhqd,bhkd->bhqk", q, k) * scale
        p = _softmax(scores, axis=-1)
        o = jnp.einsum("bhqk,bhkd->bhqd", p, v)
        return (lambda x, *d: x.transpose(*d))(o, 0, 2, 1, 3).reshape(B, S, D) @ wo

    def _B_ref(x, w1, w2):
        h = jnp.einsum("bsd,df->bsf", x, w1)
        zero = jnp.zeros_like(h)
        h = jnp.maximum(h, zero)
        return jnp.einsum("bsf,fd->bsd", h, w2)

    x = A_x
    g = _sigmoid((x * gate_w).sum(-1, keepdims=True))
    a = _A_ref(x, A_wqkv, A_wo)
    b = _B_ref(x, B_w1, B_w2)
    return g * a + (1 - g) * b
```

```python
import functools
import math

import jax
import jax.numpy as jnp
from jax import lax
import jax.experimental.pallas as pl
import jax.experimental.pallas.tpu as pltpu

S = 2048
D = 640
H = 32
DH = 20
F = 1536
LANES = 128
NT_BASE = D // LANES
NT_EXT = NT_BASE + 4
TQ = 512
CK = 128
NQ = S // TQ
NC = S // CK
VW = 24

_NT = (((1,), (1,)), ((), ()))
_TN = (((0,), (0,)), ((), ()))
_F32 = jnp.float32
_BF16 = jnp.bfloat16


def _kernel(x_ref, wqkv_ref, wo_ref, w1_ref, w2_ref, gw_ref, out_ref,
            kx_ref, qx_ref, vw_ref, sa_ref, sb_ref, ot_ref, m_ref, z_ref):
    t = pl.program_id(0)
    qscale = (DH ** -0.5) * math.log2(math.e)

    def head_q(h, tq):
        c0 = h * DH
        base = c0 // LANES
        lo = c0 % LANES
        kt = jnp.where(lo > LANES - DH, NT_BASE + base, base)
        lane = lax.broadcasted_iota(jnp.int32, (TQ, LANES), 1)
        mask = ((lane - lo) & (LANES - 1)) < DH
        q = qx_ref[kt, pl.ds(pl.multiple_of(tq * TQ, TQ), TQ), :]
        return jnp.where(mask, q, 0.0).astype(_BF16), kt

    def qk_chunk(c, qn, kt, s_w, zw):
        rows = pl.ds(c * CK, CK)
        s = lax.dot_general(kx_ref[kt, rows, :], qn, _NT, preferred_element_type=_F32)
        s_w[zw, rows, :] = s
        return jnp.max(s.reshape(CK // 8, 8, TQ), axis=0)

    @pl.when(t == 0)
    def _prologue():
        z_ref[0] = 0
        z_ref[1] = 0
        lane = lax.broadcasted_iota(jnp.int32, (TQ, LANES), 1)
        hi = lane >= 64
        for r in range(NQ):
            rows = pl.ds(r * TQ, TQ)
            xr = x_ref[rows, :]
            q = jnp.dot(xr, wqkv_ref[:, 0:D], preferred_element_type=_F32) * qscale
            k = jnp.dot(xr, wqkv_ref[:, D:2 * D], preferred_element_type=_F32)
            for j in range(NT_BASE):
                qx_ref[j, rows, :] = q[:, j * LANES:(j + 1) * LANES]
                kx_ref[j, rows, :] = k[:, j * LANES:(j + 1) * LANES].astype(_BF16)
            for e in range(4):
                qx_ref[NT_BASE + e, rows, :] = jnp.where(
                    hi, q[:, e * LANES:(e + 1) * LANES], q[:, (e + 1) * LANES:(e + 2) * LANES])
                kx_ref[NT_BASE + e, rows, :] = jnp.where(
                    hi, k[:, e * LANES:(e + 1) * LANES],
                    k[:, (e + 1) * LANES:(e + 2) * LANES]).astype(_BF16)
        wvt = wqkv_ref[:, 2 * D:3 * D].astype(_F32).T
        row = lax.broadcasted_iota(jnp.int32, (VW, TQ), 0)
        for r in range(NQ):
            cols = pl.ds(r * TQ, TQ)
            vt = lax.dot_general(wvt, x_ref[cols, :], _NT, preferred_element_type=_F32)
            for h in range(H):
                start = (h * DH) // 8 * 8
                ones_row = VW - 1 if h % 2 == 0 else 0
                vw_ref[h, :, cols] = jnp.where(row == ones_row, 1.0, vt[start:start + VW, :])
        qn, kt = head_q(0, 0)
        m8 = None
        for c in range(NC):
            cm = qk_chunk(c, qn, kt, sa_ref, 0)
            m8 = cm if m8 is None else jnp.maximum(m8, cm)
        m_ref[...] = jnp.max(m8, axis=0, keepdims=True)

    def stage(h_cur, h_nxt, tq_nxt, s_w, s_r, m_r, zw, zr):
        qn, kt = head_q(h_nxt, tq_nxt)
        m8 = None
        o = None
        for c in range(NC):
            cm = qk_chunk(c, qn, kt, s_w, zw)
            m8 = cm if m8 is None else jnp.maximum(m8, cm)
            rows = pl.ds(c * CK, CK)
            p = jnp.exp2(s_r[zr, rows, :] - m_r).astype(_BF16)
            oc = jnp.dot(vw_ref[h_cur, :, rows], p, preferred_element_type=_F32)
            o = oc if o is None else o + oc
        return jnp.max(m8, axis=0, keepdims=True), o

    def body(i, m):
        zw = z_ref[0]
        zr = z_ref[1]
        h0 = 2 * i
        m1, oe = stage(h0, h0 + 1, t, sb_ref, sa_ref, m, zw, zr)
        last = i == H // 2 - 1
        h2 = jnp.where(last, 0, h0 + 2)
        t2 = jnp.where(last, jnp.minimum(t + 1, NQ - 1), t)
        m2, oo = stage(h0 + 1, h2, t2, sa_ref, sb_ref, m1, zw, zr)
        oe = oe * (1.0 / oe[VW - 1:VW, :])
        oo = oo * (1.0 / oo[0:1, :])
        sub = lax.broadcasted_iota(jnp.int32, (8, TQ), 0)
        mid = jnp.where(sub < 4, oe[16:24, :], oo[0:8, :])
        base = pl.multiple_of(i * 40, 8)
        ot_ref[pl.ds(base, 16), :] = oe[0:16, :]
        ot_ref[pl.ds(base + 16, 8), :] = mid
        ot_ref[pl.ds(base + 24, 16), :] = oo[8:24, :]
        return m2

    m_ref[...] = lax.fori_loop(0, H // 2, body, m_ref[...])

    xt = x_ref[pl.ds(pl.multiple_of(t * TQ, TQ), TQ), :]
    a = jnp.dot(ot_ref[...].T.astype(_BF16), wo_ref[...], preferred_element_type=_F32)
    hid = jnp.maximum(jnp.dot(xt, w1_ref[...], preferred_element_type=_F32), 0.0)
    b = jnp.dot(hid.astype(_BF16), w2_ref[...], preferred_element_type=_F32)
    gl = jnp.sum(xt.astype(_F32) * gw_ref[...].astype(_F32), axis=-1, keepdims=True)
    g = 1.0 / (1.0 + jnp.exp(-gl))
    out_ref[...] = (g * a + (1.0 - g) * b).astype(out_ref.dtype)


@jax.jit
def pallas_gated_mix__softmax_full_mha__dense_activation_relu__prompt_kernel(
    A_x: jax.Array,
    A_wqkv: jax.Array,
    A_wo: jax.Array,
    B_x: jax.Array,
    B_w1: jax.Array,
    B_w2: jax.Array,
    gate_w: jax.Array,
):
    del B_x
    x = A_x.reshape(S, D)
    gw = gate_w.reshape(1, D)
    full = lambda shape: pl.BlockSpec(shape, lambda t: (0,) * len(shape))
    out = pl.pallas_call(
        _kernel,
        grid=(NQ,),
        in_specs=[full((S, D)), full((D, 3 * D)), full((D, D)), full((D, F)),
                  full((F, D)), full((1, D))],
        out_specs=pl.BlockSpec((TQ, D), lambda t: (t, 0)),
        out_shape=jax.ShapeDtypeStruct((S, D), A_x.dtype),
        scratch_shapes=[
            pltpu.VMEM((NT_EXT, S, LANES), _BF16),
            pltpu.VMEM((NT_EXT, S, LANES), _F32),
            pltpu.VMEM((H, VW, S), _F32),
            pltpu.VMEM((1, S, TQ), _F32),
            pltpu.VMEM((1, S, TQ), _F32),
            pltpu.VMEM((D, TQ), _F32),
            pltpu.VMEM((1, TQ), _F32),
            pltpu.SMEM((2,), jnp.int32),
        ],
        compiler_params=pltpu.CompilerParams(
            dimension_semantics=("arbitrary",),
            vmem_limit_bytes=100 * 1024 * 1024,
        ),
    )(x, A_wqkv, A_wo, B_w1, B_w2, gw)
    return out.reshape(1, S, D)
```

```python
import math

import jax
import jax.numpy as jnp
from jax import lax
import jax.experimental.pallas as pl
import jax.experimental.pallas.tpu as pltpu

S = 2048
D = 640
H = 32
DH = 20
F = 1536
LANES = 128
NT_BASE = D // LANES
NT_EXT = NT_BASE + 4
RC = 512
NR = S // RC
TQ = 128
NS = S // TQ
CK = 512
NC = S // CK
LAG = 2
NB = 4
VW = 24
FR = S // H
RV = 288
G = RV // 8
NBLK = 2
A = G // NBLK
SM = S - RV
KMODE = 2

_NT = (((1,), (1,)), ((), ()))
_F32 = jnp.float32
_BF16 = jnp.bfloat16
_U32 = jnp.uint32


def _kernel(x_hbm, wqkv_hbm, wo_hbm, w1_hbm, w2_hbm, gw_ref, out_hbm,
            x_ref, wqkv_ref, wo_ref, w1_ref, w2_ref, o_ref,
            w1u_ref, w2u_ref, kx_ref, kf_ref, qt_ref, vw_ref, ot_ref, b_ref, hid_ref,
            kba_ref, kbb_ref, z_ref, sem, *sbuf):
    qscale = (DH ** -0.5) * math.log2(math.e)

    def x_copy(r):
        rows = pl.ds(r * RC, RC)
        return pltpu.make_async_copy(x_hbm.at[rows, :], x_ref.at[rows, :], sem.at[r])

    def w_copy(j):
        cols = pl.ds(j * D, D)
        return pltpu.make_async_copy(wqkv_hbm.at[:, cols], wqkv_ref.at[:, cols], sem.at[NR + j])

    w1_copy = pltpu.make_async_copy(w1_hbm, w1_ref, sem.at[NR + 3])
    w2_copy = pltpu.make_async_copy(w2_hbm, w2_ref, sem.at[NR + 4])
    wo_copy = pltpu.make_async_copy(wo_hbm, wo_ref, sem.at[NR + 5])

    def out_copy(r):
        rows = pl.ds(r * RC, RC)
        return pltpu.make_async_copy(o_ref.at[rows, :], out_hbm.at[rows, :], sem.at[NR + 6 + r])

    order = [NR - 1] + list(range(NR - 1))
    w_copy(1).start()
    for r in order:
        x_copy(r).start()
    w_copy(0).start()
    w_copy(2).start()
    w1_copy.start()
    w2_copy.start()
    wo_copy.start()

    for j in range(4):
        z_ref[j] = 0
    for j in range(NB - LAG, NB):
        sbuf[j][...] = jnp.zeros_like(sbuf[j])

    hi = lax.broadcasted_iota(jnp.int32, (RC, LANES), 1) >= 64

    def kproj(r):
        y = jnp.dot(x_ref[pl.ds(r * RC, RC), :], wqkv_ref[:, D:2 * D], preferred_element_type=_F32)
        for j in range(NT_EXT):
            if j < NT_BASE:
                t = y[:, j * LANES:(j + 1) * LANES]
            else:
                e = j - NT_BASE
                t = jnp.where(hi, y[:, e * LANES:(e + 1) * LANES], y[:, (e + 1) * LANES:(e + 2) * LANES])
            t = t.astype(_BF16)
            kx_ref[j, pl.ds(r * RC // 2, RC // 2), :] = pltpu.bitcast(t, _U32)
            if r == NR - 1:
                kf_ref[j] = t[RC - RV:, :].astype(_F32)

    def head_tile(c0):
        base = c0 // LANES
        lo = c0 % LANES
        st = (lo > LANES - DH).astype(jnp.int32)
        return base, lo, st

    w_copy(1).wait()
    x_copy(order[0]).wait()
    kproj(order[0])
    for r in order[1:]:
        x_copy(r).wait()
    w_copy(0).wait()
    w_copy(2).wait()
    for r in order[1:]:
        kproj(r)
    for d in range(DH):
        kba_ref[0, d] = jnp.broadcast_to(kf_ref[0][:, d:d + 1], (RV, LANES))
    wqt = wqkv_ref[:, 0:D].astype(_F32).T
    wvt = wqkv_ref[:, 2 * D:3 * D].astype(_F32).T
    row_rc = lax.broadcasted_iota(jnp.int32, (VW, RC), 0)
    for r in range(NR):
        cols = pl.ds(r * RC, RC)
        xr = x_ref[cols, :]
        qt = lax.dot_general(wqt, xr, _NT, preferred_element_type=_F32) * qscale
        qt = qt.astype(_BF16).astype(_F32)
        for j in range(RC // TQ):
            qt_ref[r * (RC // TQ) + j] = qt[:, j * TQ:(j + 1) * TQ]
        vt = lax.dot_general(wvt, xr, _NT, preferred_element_type=_F32)
        for h in range(H):
            start = (h * DH) // 8 * 8
            ones_row = VW - 1 if h % 2 == 0 else 0
            vw_ref[h, :, cols] = jnp.where(row_rc == ones_row, 1.0, vt[start:start + VW, :])
        if r == 1:
            w1_copy.wait()
            w2_copy.wait()
            wo_copy.wait()
            w1u_ref[...] = pltpu.bitcast(w1_ref[...], _U32)
            w2u_ref[...] = pltpu.bitcast(w2_ref[...], _U32)

    row_vw = lax.broadcasted_iota(jnp.int32, (VW, TQ), 0)
    row_q = lax.broadcasted_iota(jnp.int32, (LANES, TQ), 0)

    def finish_head(h, odd, u, o):
        off = 4 if odd else 0
        ws = pl.multiple_of(h * DH - off, 8)
        l = o[0:1, :] if odd else o[VW - 1:VW, :]
        valid = (row_vw >= off) if odd else (row_vw < DH)
        pltpu.store(ot_ref.at[pl.ds(ws, VW), pl.ds(u * TQ, TQ)], o * (1.0 / l), mask=valid)

    def pv_chunk(c, h, s_r, m_r, zr):
        rows = pl.ds(c * CK, CK)
        p = jnp.exp2(s_r[zr, rows, :] - m_r)
        return jnp.dot(vw_ref[h, :, rows], p, preferred_element_type=_F32)

    def head_body(h, ms, odd):
        kb_use, kb_bld = (kbb_ref, kba_ref) if odd else (kba_ref, kbb_ref)
        zw = z_ref[0]
        zr = z_ref[1]
        never = z_ref[2] == 1
        zk = z_ref[3]
        ms = list(ms)
        c0 = (h * DH) % 1000
        base, lo, st = head_tile(c0)
        kt = base + st * NT_BASE
        lowbase = pl.multiple_of((base + st) * LANES, LANES)
        upbase = pl.multiple_of(base * LANES + 64, 64)
        rowmask = ((row_q - lo) & (LANES - 1)) < DH
        off = 4 if odd else 0
        hprev = h - 1 if odd else jnp.maximum(h - 1, 1)
        base_n, lo_n, st_n = head_tile(jnp.minimum(h + 1, H - 1) * DH)
        kt_n = base_n + st_n * NT_BASE
        shift_n = (LANES - lo_n) % LANES
        frows = pl.ds(pl.multiple_of(h * FR, FR), FR)

        def vpu_block(u, r0, s_w):
            win = qt_ref[u, pl.ds(pl.multiple_of((c0 // 8) * 8, 8), VW), :]
            accs = [None] * A
            for d in range(DH):
                qb = jnp.broadcast_to(win[off + d:off + d + 1, :], (8, LANES))
                for a in range(A):
                    t = kb_use[0, d, pl.ds((r0 + a) * 8, 8), :] * qb
                    accs[a] = t if d == 0 else accs[a] + t
            mm = None
            for a in range(A):
                s_w[zw, pl.ds(SM + (r0 + a) * 8, 8), :] = accs[a]
                mm = accs[a] if mm is None else jnp.maximum(mm, accs[a])
            return mm

        kr = None
        for u in range(NS):
            s_w = sbuf[u % NB]
            s_r = sbuf[(u - LAG) % NB]
            m_r = ms.pop(0)
            hp, podd = (h, odd) if u >= LAG else (hprev, not odd)
            if KMODE == 2:
                gb, db = u // 4, u % 4
                grows = pl.ds(gb * (RV // 4), RV // 4)
                if db == 0:
                    src = jnp.where(never, m_r, kf_ref[kt_n, grows, :])
                    kr = pltpu.roll(src, shift_n, 1)
                for d in range(db * 5, db * 5 + 5):
                    kb_bld[zk, d, grows, :] = jnp.broadcast_to(kr[:, d:d + 1], (RV // 4, LANES))
            else:
                if u == 0:
                    kr = pltpu.roll(kf_ref[kt_n], shift_n, 1)
                todo = [(d, gg) for d in range(DH) for gg in range(G)]
                for (d, gg) in todo[u * len(todo) // NS:(u + 1) * len(todo) // NS]:
                    kb_bld[zk, d, pl.ds(gg * 8, 8), :] = jnp.broadcast_to(
                        kr[gg * 8:gg * 8 + 8, d:d + 1], (8, LANES))
            qwin = jnp.concatenate(
                [qt_ref[u, pl.ds(lowbase, 64), :], qt_ref[u, pl.ds(upbase, 64), :]], axis=0)
            qn = jnp.where(rowmask, qwin, 0.0).astype(_BF16)
            m8 = None
            o = None
            done = 0
            for c in range(NC):
                n = min(CK, SM - c * CK)
                kc = pltpu.bitcast(kx_ref[kt, pl.ds(c * CK // 2, n // 2), :], _BF16)
                s = jnp.dot(kc, qn, preferred_element_type=_F32)
                s_w[zw, pl.ds(c * CK, n), :] = s
                cm = jnp.max(s.reshape(n // 8, 8, TQ), axis=0)
                m8 = cm if m8 is None else jnp.maximum(m8, cm)
                oc = pv_chunk(c, hp, s_r, m_r, zr)
                o = oc if o is None else o + oc
                upto = (c + 1) * NBLK // NC
                for blk in range(done, upto):
                    m8 = jnp.maximum(m8, vpu_block(u, blk * A, s_w))
                done = upto
            finish_head(hp, podd, (u - LAG) % NS, o)
            ms.append(jnp.max(m8, axis=0, keepdims=True))
            if u < 6:
                cols = pl.ds(u * 256, 256)
                hid = jnp.dot(x_ref[frows, :], pltpu.bitcast(w1u_ref[:, cols], _BF16),
                              preferred_element_type=_F32)
                hid_ref[zk, :, cols] = pltpu.bitcast(jnp.maximum(hid, 0.0).astype(_BF16), _U32)
            elif 8 <= u < 13:
                cols = pl.ds((u - 8) * LANES, LANES)
                b_ref[frows, cols] = jnp.dot(
                    pltpu.bitcast(hid_ref[0], _BF16), pltpu.bitcast(w2u_ref[:, cols], _BF16),
                    preferred_element_type=_F32)
        return tuple(ms)

    def body(h, ms):
        return lax.cond(h % 2 == 0,
                        lambda m: head_body(h, m, False),
                        lambda m: head_body(h, m, True), ms)

    ms = lax.fori_loop(0, H, body, tuple(jnp.zeros((1, TQ), _F32) for _ in range(LAG)))

    for j in range(LAG):
        u = NS - LAG + j
        o = None
        for c in range(NC):
            oc = pv_chunk(c, H - 1, sbuf[u % NB], ms[j], 0)
            o = oc if o is None else o + oc
        finish_head(H - 1, True, u, o)

    gw = gw_ref[...].astype(_F32)
    for r in range(NR):
        rows = pl.ds(r * RC, RC)
        a = jnp.dot(ot_ref[:, rows].T.astype(_BF16), wo_ref[...], preferred_element_type=_F32)
        b = b_ref[rows, :]
        gl = jnp.sum(x_ref[rows, :].astype(_F32) * gw, axis=-1, keepdims=True)
        g = 1.0 / (1.0 + jnp.exp(-gl))
        o_ref[rows, :] = (g * a + (1.0 - g) * b).astype(o_ref.dtype)
        out_copy(r).start()
    for r in range(NR):
        out_copy(r).wait()


@jax.jit
def pallas_gated_mix__softmax_full_mha__dense_activation_relu__prompt_kernel(
    A_x: jax.Array,
    A_wqkv: jax.Array,
    A_wo: jax.Array,
    B_x: jax.Array,
    B_w1: jax.Array,
    B_w2: jax.Array,
    gate_w: jax.Array,
):
    del B_x
    x = A_x.reshape(S, D)
    gw = gate_w.reshape(1, D)
    hbm = pl.BlockSpec(memory_space=pl.ANY)
    out = pl.pallas_call(
        _kernel,
        in_specs=[hbm, hbm, hbm, hbm, hbm, pl.BlockSpec(memory_space=pltpu.VMEM)],
        out_specs=hbm,
        out_shape=jax.ShapeDtypeStruct((S, D), A_x.dtype),
        scratch_shapes=[
            pltpu.VMEM((S, D), _BF16),
            pltpu.VMEM((D, 3 * D), _BF16),
            pltpu.VMEM((D, D), _BF16),
            pltpu.VMEM((D, F), _BF16),
            pltpu.VMEM((F, D), _BF16),
            pltpu.VMEM((S, D), _BF16),
            pltpu.VMEM((D // 2, F), _U32),
            pltpu.VMEM((F // 2, D), _U32),
            pltpu.VMEM((NT_EXT, S // 2, LANES), _U32),
            pltpu.VMEM((NT_EXT, RV, LANES), _F32),
            pltpu.VMEM((NS, D, TQ), _F32),
            pltpu.VMEM((H, VW, S), _F32),
            pltpu.VMEM((D, S), _F32),
            pltpu.VMEM((S, D), _F32),
            pltpu.VMEM((1, FR // 2, F), _U32),
            pltpu.VMEM((1, DH, RV, LANES), _F32),
            pltpu.VMEM((1, DH, RV, LANES), _F32),
            pltpu.SMEM((4,), jnp.int32),
            pltpu.SemaphoreType.DMA((2 * NR + 6,)),
        ] + [pltpu.VMEM((1, S, TQ), _F32) for _ in range(NB)],
        compiler_params=pltpu.CompilerParams(
            vmem_limit_bytes=100 * 1024 * 1024,
        ),
    )(x, A_wqkv, A_wo, B_w1, B_w2, gw)
    return out.reshape(1, S, D)
```

```python
import math

import jax
import jax.numpy as jnp
from jax import lax
import jax.experimental.pallas as pl
import jax.experimental.pallas.tpu as pltpu

S = 2048
D = 640
H = 32
DH = 20
F = 1536
LANES = 128
NT_BASE = D // LANES
NT_EXT = NT_BASE + 4
RC = 512
NR = S // RC
TQ = 128
NS = S // TQ
CK = 512
NC = S // CK
LAG = 2
NB = 4
VW = 24
FR = S // H
RV = 288
NBLK = 2
A = RV // 8 // NBLK
SM = S - RV
XSEG = ((1728, 2048), (1280, 1728), (0, 1280))
OSEG = ((0, 512), (512, 1024), (1024, 1536), (1536, 1792), (1792, 1920), (1920, 2048))
F_AFTER = {-1: (0,), 0: (1,), 1: (2,), 2: (3,), 3: (4,), 4: (5,),
           8: (6,), 9: (7,), 10: (8,), 11: (9,), 12: (10,)}

_NT = (((1,), (1,)), ((), ()))
_F32 = jnp.float32
_BF16 = jnp.bfloat16
_U32 = jnp.uint32


def _kernel(x_hbm, wqkv_hbm, wo_hbm, w1_hbm, w2_hbm, gw_hbm, out_hbm,
            x_ref, wqkv_ref, wo_ref, w1_ref, w2_ref, o_ref,
            w1u_ref, w2u_ref, kx_ref, kf_ref, qt_ref, vw_ref, ot_ref, b_ref, hid_ref,
            kba_ref, kbb_ref, z_ref, sem, *bufs):
    sbuf, gw_ref = bufs[:NB], bufs[NB]
    qscale = (DH ** -0.5) * math.log2(math.e)

    def x_copy(i):
        lo_, hi_ = XSEG[i]
        rows = pl.ds(lo_, hi_ - lo_)
        return pltpu.make_async_copy(x_hbm.at[rows, :], x_ref.at[rows, :], sem.at[i])

    def w_copy(j):
        cols = pl.ds(j * D, D)
        return pltpu.make_async_copy(wqkv_hbm.at[:, cols], wqkv_ref.at[:, cols], sem.at[3 + j])

    w1_copy = pltpu.make_async_copy(w1_hbm, w1_ref, sem.at[6])
    w2_copy = pltpu.make_async_copy(w2_hbm, w2_ref, sem.at[7])
    wo_copy = pltpu.make_async_copy(wo_hbm, wo_ref, sem.at[8])
    gw_copy = pltpu.make_async_copy(gw_hbm, gw_ref, sem.at[9])

    def out_copy(i):
        lo_, hi_ = OSEG[i]
        rows = pl.ds(lo_, hi_ - lo_)
        return pltpu.make_async_copy(o_ref.at[rows, :], out_hbm.at[rows, :], sem.at[10 + i])

    gw_copy.start()
    w_copy(1).start()
    for i in range(len(XSEG)):
        x_copy(i).start()
    w_copy(0).start()
    w_copy(2).start()
    w1_copy.start()
    w2_copy.start()
    wo_copy.start()

    for j in range(4):
        z_ref[j] = 0
    for j in range(NB - LAG, NB):
        sbuf[j][...] = jnp.zeros_like(sbuf[j])

    def kproj(r0, n):
        hi = lax.broadcasted_iota(jnp.int32, (n, LANES), 1) >= 64
        y = jnp.dot(x_ref[pl.ds(r0, n), :], wqkv_ref[:, D:2 * D], preferred_element_type=_F32)
        for j in range(NT_EXT):
            if j < NT_BASE:
                t = y[:, j * LANES:(j + 1) * LANES]
            else:
                e = j - NT_BASE
                t = jnp.where(hi, y[:, e * LANES:(e + 1) * LANES],
                              y[:, (e + 1) * LANES:(e + 2) * LANES])
            t = t.astype(_BF16)
            kx_ref[j, pl.ds(r0 // 2, n // 2), :] = pltpu.bitcast(t, _U32)
            if r0 + n > SM:
                skip = max(SM - r0, 0)
                kf_ref[j, pl.ds(r0 + skip - SM, n - skip), :] = t[skip:, :].astype(_F32)

    def head_tile(c0):
        base = c0 // LANES
        lo = c0 % LANES
        st = (lo > LANES - DH).astype(jnp.int32)
        return base, lo, st

    gw_copy.wait()
    w_copy(1).wait()
    gw = gw_ref[...].astype(_F32).reshape(1, D)
    for i, (lo_, hi_) in enumerate(XSEG):
        x_copy(i).wait()
        n = (hi_ - lo_) // 4
        for j in range(4):
            kproj(lo_ + j * n, n)
    w_copy(0).wait()
    w_copy(2).wait()
    for d in range(DH):
        kba_ref[0, d] = jnp.broadcast_to(kf_ref[0][:, d:d + 1], (RV, LANES))
    wqt = wqkv_ref[:, 0:D].astype(_F32).T.astype(_BF16)
    wvt = wqkv_ref[:, 2 * D:3 * D].astype(_F32).T.astype(_BF16)
    row_rc = lax.broadcasted_iota(jnp.int32, (VW, RC), 0)
    for r in range(NR):
        cols = pl.ds(r * RC, RC)
        xr = x_ref[cols, :]
        qt = lax.dot_general(wqt, xr, _NT, preferred_element_type=_F32) * qscale
        qt = qt.astype(_BF16).astype(_F32)
        for j in range(RC // TQ):
            qt_ref[r * (RC // TQ) + j] = qt[:, j * TQ:(j + 1) * TQ]
        vt = lax.dot_general(wvt, xr, _NT, preferred_element_type=_F32)
        for h in range(H):
            start = (h * DH) // 8 * 8
            ones_row = VW - 1 if h % 2 == 0 else 0
            vw_ref[h, :, cols] = jnp.where(row_rc == ones_row, 1.0, vt[start:start + VW, :])
        if r == 1:
            w1_copy.wait()
            w2_copy.wait()
            wo_copy.wait()
            w1u_ref[...] = pltpu.bitcast(w1_ref[...], _U32)
            w2u_ref[...] = pltpu.bitcast(w2_ref[...], _U32)

    row_vw = lax.broadcasted_iota(jnp.int32, (VW, TQ), 0)
    row_q = lax.broadcasted_iota(jnp.int32, (LANES, TQ), 0)

    def finish_head(h, odd, u, o):
        off = 4 if odd else 0
        ws = pl.multiple_of(h * DH - off, 8)
        l = o[0:1, :] if odd else o[VW - 1:VW, :]
        valid = (row_vw >= off) if odd else (row_vw < DH)
        pltpu.store(ot_ref.at[pl.ds(ws, VW), pl.ds(u * TQ, TQ)], o * (1.0 / l), mask=valid)

    def pv_chunk(c, h, j, m_r, zr):
        rows = pl.ds(c * CK, CK)
        p = jnp.exp2(sbuf[j][zr, rows, :] - m_r)
        return jnp.dot(vw_ref[h, :, rows], p, preferred_element_type=_F32)

    def head_body(h, ms, odd):
        kb_use, kb_bld = (kbb_ref, kba_ref) if odd else (kba_ref, kbb_ref)
        zw = z_ref[0]
        zr = z_ref[1]
        never = z_ref[2] == 1
        zk = z_ref[3]
        ms = list(ms)
        c0 = (h * DH) % 1000
        base, lo, st = head_tile(c0)
        kt = base + st * NT_BASE
        lowbase = pl.multiple_of((base + st) * LANES, LANES)
        upbase = pl.multiple_of(base * LANES + 64, 64)
        rowmask = ((row_q - lo) & (LANES - 1)) < DH
        off = 4 if odd else 0
        hprev = h - 1 if odd else jnp.maximum(h - 1, 1)
        base_n, lo_n, st_n = head_tile(jnp.minimum(h + 1, H - 1) * DH)
        kt_n = base_n + st_n * NT_BASE
        shift_n = (LANES - lo_n) % LANES
        frows = pl.ds(pl.multiple_of(h * FR, FR), FR)

        def vpu_block(u, r0, s_w):
            win = qt_ref[u, pl.ds(pl.multiple_of((c0 // 8) * 8, 8), VW), :]
            accs = [None] * A
            for d in range(DH):
                qb = jnp.broadcast_to(win[off + d:off + d + 1, :], (8, LANES))
                for a in range(A):
                    t = kb_use[0, d, pl.ds((r0 + a) * 8, 8), :] * qb
                    accs[a] = t if d == 0 else accs[a] + t
            mm = None
            for a in range(A):
                s_w[zw, pl.ds(SM + (r0 + a) * 8, 8), :] = accs[a]
                mm = accs[a] if mm is None else jnp.maximum(mm, accs[a])
            return mm

        def ffn_piece(j):
            if j < 6:
                cols = pl.ds(j * 256, 256)
                hid = jnp.dot(x_ref[frows, :], pltpu.bitcast(w1u_ref[:, cols], _BF16),
                              preferred_element_type=_F32)
                hid_ref[zk, :, cols] = pltpu.bitcast(jnp.maximum(hid, 0.0).astype(_BF16), _U32)
            else:
                cols = pl.ds((j - 6) * LANES, LANES)
                b_ref[frows, cols] = jnp.dot(
                    pltpu.bitcast(hid_ref[0], _BF16), pltpu.bitcast(w2u_ref[:, cols], _BF16),
                    preferred_element_type=_F32)

        kr = None
        for j in F_AFTER.get(-1, ()):
            ffn_piece(j)
        for u in range(NS):
            s_w = sbuf[u % NB]
            m_r = ms.pop(0)
            hp, podd = (h, odd) if u >= LAG else (hprev, not odd)
            gb, db = u // 4, u % 4
            grows = pl.ds(gb * (RV // 4), RV // 4)
            if db == 0:
                src = jnp.where(never, m_r, kf_ref[kt_n, grows, :])
                kr = pltpu.roll(src, shift_n, 1)
            for d in range(db * 5, db * 5 + 5):
                kb_bld[zk, d, grows, :] = jnp.broadcast_to(kr[:, d:d + 1], (RV // 4, LANES))
            qwin = jnp.concatenate(
                [qt_ref[u, pl.ds(lowbase, 64), :], qt_ref[u, pl.ds(upbase, 64), :]], axis=0)
            qn = jnp.where(rowmask, qwin, 0.0).astype(_BF16)
            m8 = None
            o = None
            done = 0
            for c in range(NC):
                n = min(CK, SM - c * CK)
                kc = pltpu.bitcast(kx_ref[kt, pl.ds(c * CK // 2, n // 2), :], _BF16)
                s = jnp.dot(kc, qn, preferred_element_type=_F32)
                s_w[zw, pl.ds(c * CK, n), :] = s
                cm = jnp.max(s.reshape(n // 8, 8, TQ), axis=0)
                m8 = cm if m8 is None else jnp.maximum(m8, cm)
                oc = pv_chunk(c, hp, (u - LAG) % NB, m_r, zr)
                o = oc if o is None else o + oc
                upto = (c + 1) * NBLK // NC
                for blk in range(done, upto):
                    m8 = jnp.maximum(m8, vpu_block(u, blk * A, s_w))
                done = upto
            finish_head(hp, podd, (u - LAG) % NS, o)
            ms.append(jnp.max(m8, axis=0, keepdims=True))
            for j in F_AFTER.get(u, ()):
                ffn_piece(j)
        return tuple(ms)

    def body(h, ms):
        return lax.cond(h % 2 == 0,
                        lambda m: head_body(h, m, False),
                        lambda m: head_body(h, m, True), ms)

    ms = lax.fori_loop(0, H, body, tuple(jnp.zeros((1, TQ), _F32) for _ in range(LAG)))

    for j in range(LAG):
        u = NS - LAG + j
        o = None
        for c in range(NC):
            oc = pv_chunk(c, H - 1, u % NB, ms[j], 0)
            o = oc if o is None else o + oc
        finish_head(H - 1, True, u, o)

    for i, (lo_, hi_) in enumerate(OSEG):
        rows = pl.ds(lo_, hi_ - lo_)
        a = jnp.dot(ot_ref[:, rows].T.astype(_BF16), wo_ref[...], preferred_element_type=_F32)
        b = b_ref[rows, :]
        gl = jnp.sum(x_ref[rows, :].astype(_F32) * gw, axis=-1, keepdims=True)
        g = 1.0 / (1.0 + jnp.exp(-gl))
        o_ref[rows, :] = (g * a + (1.0 - g) * b).astype(o_ref.dtype)
        out_copy(i).start()
    for i in range(len(OSEG)):
        out_copy(i).wait()


@jax.jit
def pallas_gated_mix__softmax_full_mha__dense_activation_relu__prompt_kernel(
    A_x: jax.Array,
    A_wqkv: jax.Array,
    A_wo: jax.Array,
    B_x: jax.Array,
    B_w1: jax.Array,
    B_w2: jax.Array,
    gate_w: jax.Array,
):
    del B_x
    x = A_x.reshape(S, D)
    hbm = pl.BlockSpec(memory_space=pl.ANY)
    out = pl.pallas_call(
        _kernel,
        in_specs=[hbm] * 6,
        out_specs=hbm,
        out_shape=jax.ShapeDtypeStruct((S, D), A_x.dtype),
        scratch_shapes=[
            pltpu.VMEM((S, D), _BF16),
            pltpu.VMEM((D, 3 * D), _BF16),
            pltpu.VMEM((D, D), _BF16),
            pltpu.VMEM((D, F), _BF16),
            pltpu.VMEM((F, D), _BF16),
            pltpu.VMEM((S, D), _BF16),
            pltpu.VMEM((D // 2, F), _U32),
            pltpu.VMEM((F // 2, D), _U32),
            pltpu.VMEM((NT_EXT, S // 2, LANES), _U32),
            pltpu.VMEM((NT_EXT, RV, LANES), _F32),
            pltpu.VMEM((NS, D, TQ), _F32),
            pltpu.VMEM((H, VW, S), _F32),
            pltpu.VMEM((D, S), _F32),
            pltpu.VMEM((S, D), _F32),
            pltpu.VMEM((1, FR // 2, F), _U32),
            pltpu.VMEM((1, DH, RV, LANES), _F32),
            pltpu.VMEM((1, DH, RV, LANES), _F32),
            pltpu.SMEM((4,), jnp.int32),
            pltpu.SemaphoreType.DMA((10 + len(OSEG),)),
        ] + [pltpu.VMEM((1, S, TQ), _F32) for _ in range(NB)]
        + [pltpu.VMEM((D,), _BF16)],
        compiler_params=pltpu.CompilerParams(
            vmem_limit_bytes=100 * 1024 * 1024,
        ),
    )(x, A_wqkv, A_wo, B_w1, B_w2, gate_w)
    return out.reshape(1, S, D)
```

```python
import math

import jax
import jax.numpy as jnp
from jax import lax
import jax.experimental.pallas as pl
import jax.experimental.pallas.tpu as pltpu

S = 2048
D = 640
H = 32
DH = 20
F = 1536
LANES = 128
NT_BASE = D // LANES
NT_EXT = NT_BASE + 4
RC = 512
NR = S // RC
TQ = 128
NS = S // TQ
CK = 512
NC = S // CK
LAG = 2
NB = 4
VW = 24
FR = S // H
RVS = (288,) * 8 + (320,) * 8
RV = max(RVS)
NBLK = 2
SM = S - RV
XSEG = ((1728, 2048), (1280, 1728), (0, 1280))
OSEG = ((0, 512), (512, 1024), (1024, 1536), (1536, 1792), (1792, 1920), (1920, 2048))
F_AFTER = {-1: (0,), 0: (1,), 1: (2,), 2: (3,), 3: (4,), 4: (5,),
           8: (6,), 9: (7,), 10: (8,), 11: (9,), 12: (10,)}

_NT = (((1,), (1,)), ((), ()))
_F32 = jnp.float32
_BF16 = jnp.bfloat16
_U32 = jnp.uint32


def _kernel(x_hbm, wqkv_hbm, wo_hbm, w1_hbm, w2_hbm, gw_hbm, out_hbm,
            x_ref, wqkv_ref, wo_ref, w1_ref, w2_ref, o_ref,
            w1u_ref, w2u_ref, kx_ref, kf_ref, qt_ref, vw_ref, ot_ref, b_ref, hid_ref,
            kba_ref, kbb_ref, z_ref, sem, *bufs):
    sbuf, gw_ref = bufs[:NB], bufs[NB]
    qscale = (DH ** -0.5) * math.log2(math.e)

    def x_copy(i):
        lo_, hi_ = XSEG[i]
        rows = pl.ds(lo_, hi_ - lo_)
        return pltpu.make_async_copy(x_hbm.at[rows, :], x_ref.at[rows, :], sem.at[i])

    def w_copy(j):
        cols = pl.ds(j * D, D)
        return pltpu.make_async_copy(wqkv_hbm.at[:, cols], wqkv_ref.at[:, cols], sem.at[3 + j])

    w1_copy = pltpu.make_async_copy(w1_hbm, w1_ref, sem.at[6])
    w2_copy = pltpu.make_async_copy(w2_hbm, w2_ref, sem.at[7])
    wo_copy = pltpu.make_async_copy(wo_hbm, wo_ref, sem.at[8])
    gw_copy = pltpu.make_async_copy(gw_hbm, gw_ref, sem.at[9])

    def out_copy(i):
        lo_, hi_ = OSEG[i]
        rows = pl.ds(lo_, hi_ - lo_)
        return pltpu.make_async_copy(o_ref.at[rows, :], out_hbm.at[rows, :], sem.at[10 + i])

    gw_copy.start()
    w_copy(1).start()
    for i in range(len(XSEG)):
        x_copy(i).start()
    w_copy(0).start()
    w_copy(2).start()
    w1_copy.start()
    w2_copy.start()
    wo_copy.start()

    for j in range(4):
        z_ref[j] = 0
    for j in range(NB - LAG, NB):
        sbuf[j][...] = jnp.zeros_like(sbuf[j])

    def kproj(r0, n):
        hi = lax.broadcasted_iota(jnp.int32, (n, LANES), 1) >= 64
        y = jnp.dot(x_ref[pl.ds(r0, n), :], wqkv_ref[:, D:2 * D], preferred_element_type=_F32)
        for j in range(NT_EXT):
            if j < NT_BASE:
                t = y[:, j * LANES:(j + 1) * LANES]
            else:
                e = j - NT_BASE
                t = jnp.where(hi, y[:, e * LANES:(e + 1) * LANES],
                              y[:, (e + 1) * LANES:(e + 2) * LANES])
            t = t.astype(_BF16)
            kx_ref[j, pl.ds(r0 // 2, n // 2), :] = pltpu.bitcast(t, _U32)
            if r0 + n > SM:
                skip = max(SM - r0, 0)
                kf_ref[j, pl.ds(r0 + skip - SM, n - skip), :] = t[skip:, :].astype(_F32)

    def head_tile(c0):
        base = c0 // LANES
        lo = c0 % LANES
        st = (lo > LANES - DH).astype(jnp.int32)
        return base, lo, st

    gw_copy.wait()
    w_copy(1).wait()
    gw = gw_ref[...].astype(_F32).reshape(1, D)
    for i, (lo_, hi_) in enumerate(XSEG):
        x_copy(i).wait()
        n = (hi_ - lo_) // 4
        for j in range(4):
            kproj(lo_ + j * n, n)
    w_copy(0).wait()
    w_copy(2).wait()
    for d in range(DH):
        kba_ref[0, d] = jnp.broadcast_to(kf_ref[0][:, d:d + 1], (RV, LANES))
    wqt = wqkv_ref[:, 0:D].astype(_F32).T.astype(_BF16)
    wvt = wqkv_ref[:, 2 * D:3 * D].astype(_F32).T.astype(_BF16)
    row_rc = lax.broadcasted_iota(jnp.int32, (VW, RC), 0)
    for r in range(NR):
        cols = pl.ds(r * RC, RC)
        xr = x_ref[cols, :]
        qt = lax.dot_general(wqt, xr, _NT, preferred_element_type=_F32) * qscale
        qt = qt.astype(_BF16).astype(_F32)
        for j in range(RC // TQ):
            qt_ref[r * (RC // TQ) + j] = qt[:, j * TQ:(j + 1) * TQ]
        vt = lax.dot_general(wvt, xr, _NT, preferred_element_type=_F32)
        for h in range(H):
            start = (h * DH) // 8 * 8
            ones_row = VW - 1 if h % 2 == 0 else 0
            vw_ref[h, :, cols] = jnp.where(row_rc == ones_row, 1.0, vt[start:start + VW, :])
        if r == 1:
            w1_copy.wait()
            w2_copy.wait()
            wo_copy.wait()
            w1u_ref[...] = pltpu.bitcast(w1_ref[...], _U32)
            w2u_ref[...] = pltpu.bitcast(w2_ref[...], _U32)

    row_vw = lax.broadcasted_iota(jnp.int32, (VW, TQ), 0)
    row_q = lax.broadcasted_iota(jnp.int32, (LANES, TQ), 0)

    def finish_head(h, odd, u, o):
        off = 4 if odd else 0
        ws = pl.multiple_of(h * DH - off, 8)
        l = o[0:1, :] if odd else o[VW - 1:VW, :]
        valid = (row_vw >= off) if odd else (row_vw < DH)
        pltpu.store(ot_ref.at[pl.ds(ws, VW), pl.ds(u * TQ, TQ)], o * (1.0 / l), mask=valid)

    def pv_chunk(c, h, j, m_r, zr):
        rows = pl.ds(c * CK, CK)
        p = jnp.exp2(sbuf[j][zr, rows, :] - m_r)
        return jnp.dot(vw_ref[h, :, rows], p, preferred_element_type=_F32)

    def head_body(h, ms, odd):
        kb_use, kb_bld = (kbb_ref, kba_ref) if odd else (kba_ref, kbb_ref)
        zw = z_ref[0]
        zr = z_ref[1]
        never = z_ref[2] == 1
        zk = z_ref[3]
        ms = list(ms)
        c0 = (h * DH) % 1000
        base, lo, st = head_tile(c0)
        kt = base + st * NT_BASE
        lowbase = pl.multiple_of((base + st) * LANES, LANES)
        upbase = pl.multiple_of(base * LANES + 64, 64)
        rowmask = ((row_q - lo) & (LANES - 1)) < DH
        off = 4 if odd else 0
        hprev = h - 1 if odd else jnp.maximum(h - 1, 1)
        base_n, lo_n, st_n = head_tile(jnp.minimum(h + 1, H - 1) * DH)
        kt_n = base_n + st_n * NT_BASE
        shift_n = (LANES - lo_n) % LANES
        frows = pl.ds(pl.multiple_of(h * FR, FR), FR)

        def vpu_block(u, r0, A, s_w):
            win = qt_ref[u, pl.ds(pl.multiple_of((c0 // 8) * 8, 8), VW), :]
            accs = [None] * A
            for d in range(DH):
                qb = jnp.broadcast_to(win[off + d:off + d + 1, :], (8, LANES))
                for a in range(A):
                    t = kb_use[0, d, pl.ds((r0 + a) * 8, 8), :] * qb
                    accs[a] = t if d == 0 else accs[a] + t
            mm = None
            for a in range(A):
                s_w[zw, pl.ds(SM + (r0 + a) * 8, 8), :] = accs[a]
                mm = accs[a] if mm is None else jnp.maximum(mm, accs[a])
            return mm

        def ffn_piece(j):
            if j < 6:
                cols = pl.ds(j * 256, 256)
                hid = jnp.dot(x_ref[frows, :], pltpu.bitcast(w1u_ref[:, cols], _BF16),
                              preferred_element_type=_F32)
                hid_ref[zk, :, cols] = pltpu.bitcast(jnp.maximum(hid, 0.0).astype(_BF16), _U32)
            else:
                cols = pl.ds((j - 6) * LANES, LANES)
                b_ref[frows, cols] = jnp.dot(
                    pltpu.bitcast(hid_ref[0], _BF16), pltpu.bitcast(w2u_ref[:, cols], _BF16),
                    preferred_element_type=_F32)

        kr0 = None
        for j in F_AFTER.get(-1, ()):
            ffn_piece(j)
        for u in range(NS):
            s_w = sbuf[u % NB]
            m_r = ms.pop(0)
            hp, podd = (h, odd) if u >= LAG else (hprev, not odd)
            gb, db = u // 4, u % 4
            grows = pl.ds(gb * (RV // 4), RV // 4)
            if db == 0:
                src = jnp.where(never, m_r, kf_ref[kt_n, grows, :])
                kr0 = pltpu.roll(src, shift_n, 1)
                kr = kr0
            else:
                kr = jnp.where(never, m_r, kr0)
            for d in range(db * 5, db * 5 + 5):
                kb_bld[zk, d, grows, :] = jnp.broadcast_to(kr[:, d:d + 1], (RV // 4, LANES))
            qwin = jnp.concatenate(
                [qt_ref[u, pl.ds(lowbase, 64), :], qt_ref[u, pl.ds(upbase, 64), :]], axis=0)
            qn = jnp.where(rowmask, qwin, 0.0).astype(_BF16)
            m8 = None
            o = None
            done = 0
            for c in range(NC):
                n = min(CK, S - RVS[u] - c * CK)
                kc = pltpu.bitcast(kx_ref[kt, pl.ds(c * CK // 2, n // 2), :], _BF16)
                s = jnp.dot(kc, qn, preferred_element_type=_F32)
                s_w[zw, pl.ds(c * CK, n), :] = s
                cm = jnp.max(s.reshape(n // 8, 8, TQ), axis=0)
                m8 = cm if m8 is None else jnp.maximum(m8, cm)
                oc = pv_chunk(c, hp, (u - LAG) % NB, m_r, zr)
                o = oc if o is None else o + oc
                upto = (c + 1) * NBLK // NC
                for blk in range(done, upto):
                    A = RVS[u] // 8 // NBLK
                    m8 = jnp.maximum(m8, vpu_block(u, (RV - RVS[u]) // 8 + blk * A, A, s_w))
                done = upto
            finish_head(hp, podd, (u - LAG) % NS, o)
            ms.append(jnp.max(m8, axis=0, keepdims=True))
            for j in F_AFTER.get(u, ()):
                ffn_piece(j)
        return tuple(ms)

    def body(h, ms):
        return lax.cond(h % 2 == 0,
                        lambda m: head_body(h, m, False),
                        lambda m: head_body(h, m, True), ms)

    ms = lax.fori_loop(0, H, body, tuple(jnp.zeros((1, TQ), _F32) for _ in range(LAG)))

    for j in range(LAG):
        u = NS - LAG + j
        o = None
        for c in range(NC):
            oc = pv_chunk(c, H - 1, u % NB, ms[j], 0)
            o = oc if o is None else o + oc
        finish_head(H - 1, True, u, o)

    for i, (lo_, hi_) in enumerate(OSEG):
        rows = pl.ds(lo_, hi_ - lo_)
        a = jnp.dot(ot_ref[:, rows].T.astype(_BF16), wo_ref[...], preferred_element_type=_F32)
        b = b_ref[rows, :]
        gl = jnp.sum(x_ref[rows, :].astype(_F32) * gw, axis=-1, keepdims=True)
        g = 1.0 / (1.0 + jnp.exp(-gl))
        o_ref[rows, :] = (g * a + (1.0 - g) * b).astype(o_ref.dtype)
        out_copy(i).start()
    for i in range(len(OSEG)):
        out_copy(i).wait()


@jax.jit
def pallas_gated_mix__softmax_full_mha__dense_activation_relu__prompt_kernel(
    A_x: jax.Array,
    A_wqkv: jax.Array,
    A_wo: jax.Array,
    B_x: jax.Array,
    B_w1: jax.Array,
    B_w2: jax.Array,
    gate_w: jax.Array,
):
    del B_x
    x = A_x.reshape(S, D)
    hbm = pl.BlockSpec(memory_space=pl.ANY)
    out = pl.pallas_call(
        _kernel,
        in_specs=[hbm] * 6,
        out_specs=hbm,
        out_shape=jax.ShapeDtypeStruct((S, D), A_x.dtype),
        scratch_shapes=[
            pltpu.VMEM((S, D), _BF16),
            pltpu.VMEM((D, 3 * D), _BF16),
            pltpu.VMEM((D, D), _BF16),
            pltpu.VMEM((D, F), _BF16),
            pltpu.VMEM((F, D), _BF16),
            pltpu.VMEM((S, D), _BF16),
            pltpu.VMEM((D // 2, F), _U32),
            pltpu.VMEM((F // 2, D), _U32),
            pltpu.VMEM((NT_EXT, S // 2, LANES), _U32),
            pltpu.VMEM((NT_EXT, RV, LANES), _F32),
            pltpu.VMEM((NS, D, TQ), _F32),
            pltpu.VMEM((H, VW, S), _F32),
            pltpu.VMEM((D, S), _F32),
            pltpu.VMEM((S, D), _F32),
            pltpu.VMEM((1, FR // 2, F), _U32),
            pltpu.VMEM((1, DH, RV, LANES), _F32),
            pltpu.VMEM((1, DH, RV, LANES), _F32),
            pltpu.SMEM((4,), jnp.int32),
            pltpu.SemaphoreType.DMA((10 + len(OSEG),)),
        ] + [pltpu.VMEM((1, S, TQ), _F32) for _ in range(NB)]
        + [pltpu.VMEM((D,), _BF16)],
        compiler_params=pltpu.CompilerParams(
            vmem_limit_bytes=100 * 1024 * 1024,
        ),
    )(x, A_wqkv, A_wo, B_w1, B_w2, gate_w)
    return out.reshape(1, S, D)
```
